```python
import os as _os
_os.environ.setdefault("JAX_PLATFORMS", "cpu")
import jax
import jax.numpy as jnp

def _softmax(x, axis=-1):
    return jax.nn.softmax(x, axis=axis)
def _gelu(x):
    return jax.nn.gelu(x, approximate=True)
def _silu(x):
    return jax.nn.silu(x)
def _sigmoid(x):
    return jax.nn.sigmoid(x)
def _layernorm(x, axis=-1, eps=1e-5):
    m = jnp.mean(x, axis=axis, keepdims=True)
    v = jnp.var(x, axis=axis, keepdims=True)
    return (x - m) / jnp.sqrt(v + eps)
def _scatter_add(tgt, idx, src, axis=0):
    return tgt.at[idx].add(src)
def _segment_sum(src, seg, n):
    return jax.ops.segment_sum(src, seg, n)
class _Rng:
    def __init__(self, key):
        self._k = key
    def _next(self):
        self._k, sub = jax.random.split(self._k)
        return sub
    def normal(self, shape):
        return jax.random.normal(self._next(), shape, dtype=jnp.bfloat16)
    def randint(self, lo, hi, shape):
        return jax.random.randint(self._next(), shape, lo, hi, dtype=jnp.int32)
    def uniform(self, shape, lo=0.0, hi=1.0):
        return jax.random.uniform(self._next(), shape, jnp.bfloat16, lo, hi)
    def permutation(self, n):
        return jax.random.permutation(self._next(), n)


kernel_name = 'standalone__gqa_block_cached__near_ridge'

def setup_inputs():
    _rng = _Rng(jax.random.key(int.from_bytes(__import__("os").urandom(4), "little")))
    _w = (lambda a: (lambda t: t.astype(jnp.bfloat16) if jnp.issubdtype(t.dtype, jnp.floating) else t)(jnp.asarray(a)))
    B, Sq, D = 8, 64, 512
    Hq, Hkv, Sk, Dh = 32, 8, 64, 128
    assert Hq % Hkv == 0, (Hq, Hkv)
    return {
        "x": _w((lambda *s: _rng.normal(s) * 0.8)(B, Sq, D)),
        "k_cache": _w((lambda *s: _rng.normal(s) * 0.8)(B, Hkv, Sk, Dh)),
        "v_cache": _w((lambda *s: _rng.normal(s) * 0.05)(B, Hkv, Sk, Dh)),
        "wq": _w((lambda *s: _rng.normal(s) * 0.8)(D, Hq * Dh) * (D ** -0.5)),
        "wo": _w((lambda *s: _rng.normal(s) * 0.05)(Hq * Dh, D) * ((Hq * Dh) ** -0.5)),
    }

def reference(x, k_cache, v_cache, wq, wo):
    B, Sq, D = x.shape
    Hq, Dh = 32, 128
    Hkv = k_cache.shape[1]
    rep = Hq // Hkv
    q = (lambda x, *d: x.transpose(*d))((x @ wq).reshape(B, Sq, Hq, Dh), 0, 2, 1, 3)
    k = jnp.repeat(k_cache, rep, axis=1)
    v = jnp.repeat(v_cache, rep, axis=1)
    scores = jnp.einsum("bhqd,bhkd->bhqk", q, k) * (Dh ** -0.5)
    p = _softmax(scores, axis=-1)
    o = jnp.einsum("bhqk,bhkd->bhqd", p, v)
    return (lambda x, *d: x.transpose(*d))(o, 0, 2, 1, 3).reshape(B, Sq, Hq * Dh) @ wo
```

```python
import jax
import jax.numpy as jnp
import jax.experimental.pallas as pl
import jax.experimental.pallas.tpu as pltpu


@jax.jit
def pallas_standalone__gqa_block_cached__near_ridge_kernel(
    x: jax.Array,
    k_cache: jax.Array,
    v_cache: jax.Array,
    wq: jax.Array,
    wo: jax.Array,
):
    B, Sq, D = x.shape
    _, Hkv, Sk, Dh = k_cache.shape
    Hq = wq.shape[1] // Dh
    rep = Hq // Hkv
    GW = rep * Dh
    M = B * Sq
    scale = Dh ** -0.5

    def kernel_function(x_ref, k_ref, v_ref, wq_ref, wo_ref, out_ref, acc_ref):
        g = pl.program_id(0)
        q = jnp.dot(x_ref[...], wq_ref[...], preferred_element_type=jnp.float32)
        q = q.astype(jnp.bfloat16)
        outs = []
        for b in range(B):
            qb = q[b * Sq:(b + 1) * Sq]
            qs = jnp.concatenate([qb[:, h * Dh:(h + 1) * Dh] for h in range(rep)], axis=0)
            s = jax.lax.dot_general(qs, k_ref[b, 0], (((1,), (1,)), ((), ())),
                                    preferred_element_type=jnp.float32)
            s = s * scale
            m = jnp.max(s, axis=-1, keepdims=True)
            e = jnp.exp(s - m)
            p = e / jnp.sum(e, axis=-1, keepdims=True)
            o = jnp.dot(p.astype(jnp.bfloat16), v_ref[b, 0], preferred_element_type=jnp.float32)
            o = o.astype(jnp.bfloat16)
            outs.append(jnp.concatenate([o[h * Sq:(h + 1) * Sq] for h in range(rep)], axis=1))
        o_all = jnp.concatenate(outs, axis=0)
        contrib = jnp.dot(o_all, wo_ref[...], preferred_element_type=jnp.float32)

        @pl.when(g == 0)
        def _():
            acc_ref[...] = contrib

        @pl.when(g > 0)
        def _():
            acc_ref[...] += contrib

        @pl.when(g == Hkv - 1)
        def _():
            out_ref[...] = acc_ref[...].astype(out_ref.dtype)

    out = pl.pallas_call(
        kernel_function,
        grid=(Hkv,),
        in_specs=[
            pl.BlockSpec((M, D), lambda g: (0, 0)),
            pl.BlockSpec((B, 1, Sk, Dh), lambda g: (0, g, 0, 0)),
            pl.BlockSpec((B, 1, Sk, Dh), lambda g: (0, g, 0, 0)),
            pl.BlockSpec((D, GW), lambda g: (0, g)),
            pl.BlockSpec((GW, D), lambda g: (g, 0)),
        ],
        out_specs=pl.BlockSpec((M, D), lambda g: (0, 0)),
        out_shape=jax.ShapeDtypeStruct((M, D), x.dtype),
        scratch_shapes=[pltpu.VMEM((M, D), jnp.float32)],
        compiler_params=pltpu.CompilerParams(
            dimension_semantics=("arbitrary",),
            vmem_limit_bytes=64 * 1024 * 1024,
        ),
    )(x.reshape(M, D), k_cache, v_cache, wq, wo)
    return out.reshape(B, Sq, D)
```

```python
import functools

import jax
import jax.numpy as jnp
import jax.experimental.pallas as pl
import jax.experimental.pallas.tpu as pltpu

_LOG2E = 1.4426950408889634
_T = 128
_NUM_SEMS = 4
_NT_DIMS = (((1,), (1,)), ((), ()))


def _copy_stages(n_kv):
    kv = lambda *names: [(n[0], int(n[1:])) for n in names]
    stages = [
        [("x", 0), ("wqk", 0, 0), ("wqk", 1, 0)],
        [("x", 1), ("wqk", 0, 1)],
        [("wqk", 1, 1)],
        [("x", 2), ("wqk", 0, 2), ("wqk", 1, 2)],
        [("x", 3), ("wqk", 0, 3), ("wqk", 1, 3)],
        [("k", 0), ("wqn", 2, 0)],
        [("wqn", 2, 1), ("wqn", 2, 2), ("wqn", 2, 3), ("v", 0)],
        kv("k1", "o0", "v1"),
        kv("q3", "k2", "o1", "v2"),
        kv("q4", "k3", "o2", "v3", "q5", "k4", "o3", "v4"),
        kv("q6", "k5", "o4", "v5", "q7", "k6", "o5", "v6", "k7", "o6", "v7", "o7"),
    ]
    assert n_kv == 8
    rename = {"q": "wq", "o": "wo"}
    return [[(rename.get(it[0], it[0]),) + tuple(it[1:]) for it in st] for st in stages]


def _schedule(n_kv):
    tasks = [("prologue",)]
    for g in range(n_kv):
        for j in range(4):
            tasks.append(("scores", g, j))
            tasks.append(("qproj", 2, j) if g == 0 else ("oproj", g - 1, j))
        if 1 <= g < n_kv - 2:
            tasks += [("pv", g, 0), ("qproj", g + 2, 0), ("qproj", g + 2, 1),
                      ("pv", g, 1), ("qproj", g + 2, 2), ("qproj", g + 2, 3)]
        else:
            tasks += [("pv", g, 0), ("pv", g, 1)]
    tasks += [("oproj", n_kv - 1, j) for j in range(4)]
    return tasks


def _gqa_block_kernel(x_hbm, k_hbm, v_hbm, wq_hbm, wo_hbm, out_hbm,
                      x_v, wq_v, wo_v, k_v, v_v, acc_v, out_v, sems,
                      *, batch, sq, n_kv, rep, dh, scale):
    f32, bf16 = jnp.float32, jnp.bfloat16
    rows = batch * sq
    gw = rep * dh
    stages = _copy_stages(n_kv)
    n_stages = len(stages)

    def copy(item, stage):
        sem = sems.at[stage % _NUM_SEMS]
        kind, g = item[0], item[1]
        if kind == "x":
            cols = pl.ds(g * _T, _T)
            return pltpu.make_async_copy(x_hbm.at[:, cols], x_v.at[:, cols], sem)
        if kind == "wqk":
            rws = pl.ds(item[2] * _T, _T)
            return pltpu.make_async_copy(
                wq_hbm.at[rws, pl.ds(g * gw, gw)], wq_v.at[g, rws, :], sem)
        if kind == "wqn":
            return pltpu.make_async_copy(
                wq_hbm.at[:, pl.ds(g * gw + item[2] * dh, dh)],
                wq_v.at[g, :, pl.ds(item[2] * dh, dh)], sem)
        if kind == "wq":
            return pltpu.make_async_copy(
                wq_hbm.at[:, pl.ds(g * gw, gw)], wq_v.at[g], sem)
        if kind == "wo":
            return pltpu.make_async_copy(
                wo_hbm.at[pl.ds(g * gw, gw), :], wo_v.at[g], sem)
        if kind == "k":
            return pltpu.make_async_copy(k_hbm.at[:, g], k_v.at[g], sem)
        assert kind == "v", kind
        return pltpu.make_async_copy(v_hbm.at[:, g], v_v.at[g], sem)

    def start_stage(s):
        for item in stages[s]:
            copy(item, s).start()

    waited = []

    def wait_through(stage):
        while len(waited) <= stage:
            s = len(waited)
            for item in stages[s]:
                copy(item, s).wait()
            waited.append(s)
            if s + _NUM_SEMS < n_stages:
                start_stage(s + _NUM_SEMS)

    stage_of = {item: s for s, st in enumerate(stages) for item in st}

    def need(*items):
        wait_through(max(stage_of[item] for item in items))

    q, p, o = {}, {}, {}
    out_copies = []

    def prologue():
        n_rb = 4
        acc = {}
        for k in range(x_v.shape[1] // _T):
            ks = slice(k * _T, (k + 1) * _T)
            need(("x", k))
            xs = [x_v[i * rows // n_rb:(i + 1) * rows // n_rb, ks] for i in range(n_rb)]
            for g in range(2):
                need(("wqk", g, k))
                part = jnp.concatenate(
                    [jnp.dot(xi, wq_v[g, ks, :], preferred_element_type=f32) for xi in xs],
                    axis=0)
                acc[g] = part if k == 0 else acc[g] + part
        for g in range(2):
            for h in range(rep):
                q[g, h] = acc[g][:, h * dh:(h + 1) * dh]

    def qproj(g, h):
        need(("wqn", g, h) if ("wqn", g, h) in stage_of else ("wq", g))
        q[g, h] = jnp.dot(x_v[...], wq_v[g, :, h * dh:(h + 1) * dh],
                          preferred_element_type=f32)

    def scores(g, j):
        need(("k", g))
        for b in (2 * j, 2 * j + 1):
            qs = jnp.concatenate(
                [q[g, h][b * sq:(b + 1) * sq] for h in range(rep)], axis=0).astype(bf16)
            st = jax.lax.dot_general(k_v[g, b], qs, _NT_DIMS,
                                     preferred_element_type=f32)
            m = jnp.max(st, axis=0, keepdims=True)
            e = jnp.exp2((st - m) * (scale * _LOG2E))
            denom = jnp.sum(e, axis=0, keepdims=True)
            p[g, b] = (e * pl.reciprocal(denom, approx=False)).astype(bf16).T

    def pv(g, half):
        need(("v", g))
        for b in range(half * batch // 2, (half + 1) * batch // 2):
            ob = jnp.dot(p.pop((g, b)), v_v[g, b], preferred_element_type=f32)
            o[g, b] = jnp.concatenate(
                [ob[h * sq:(h + 1) * sq] for h in range(rep)], axis=1)

    def oproj(g, j):
        need(("wo", g))
        if j == 0:
            o[g] = jnp.concatenate([o.pop((g, b)) for b in range(batch)], axis=0)
        cols = slice(j * _T, (j + 1) * _T)
        if g < n_kv - 1:
            part = jnp.dot(o[g].astype(bf16), wo_v[g, :, cols], preferred_element_type=f32)
            if g == 0:
                acc_v[:, cols] = part
            else:
                acc_v[:, cols] += part
            return
        wait_through(n_stages - 1)
        n_rb = 4 if j == 3 else 1
        for i in range(n_rb):
            rws = slice(i * rows // n_rb, (i + 1) * rows // n_rb)
            part = jnp.dot(o[g][rws].astype(bf16), wo_v[g, :, cols],
                           preferred_element_type=f32)
            out_v[rws, cols] = (acc_v[rws, cols] + part).astype(out_v.dtype)
            out_copy = pltpu.make_async_copy(
                out_v.at[rws, cols], out_hbm.at[rws, cols], sems.at[n_stages % _NUM_SEMS])
            out_copy.start()
            out_copies.append(out_copy)

    for s in range(_NUM_SEMS):
        start_stage(s)
    run = dict(prologue=prologue, qproj=qproj, scores=scores, pv=pv, oproj=oproj)
    for task in _schedule(n_kv):
        run[task[0]](*task[1:])
    for out_copy in out_copies:
        out_copy.wait()


@jax.jit
def pallas_standalone__gqa_block_cached__near_ridge_kernel(
    x: jax.Array,
    k_cache: jax.Array,
    v_cache: jax.Array,
    wq: jax.Array,
    wo: jax.Array,
):
    batch, sq, d_model = x.shape
    _, n_kv, sk, dh = k_cache.shape
    n_q = wq.shape[1] // dh
    rep = n_q // n_kv
    gw = rep * dh
    rows = batch * sq
    assert (batch, sq, d_model, n_kv, sk, dh, n_q) == (8, 64, 512, 8, 64, 128, 32)

    kernel = functools.partial(
        _gqa_block_kernel, batch=batch, sq=sq, n_kv=n_kv, rep=rep, dh=dh,
        scale=dh ** -0.5)
    out = pl.pallas_call(
        kernel,
        in_specs=[pl.BlockSpec(memory_space=pl.ANY)] * 5,
        out_specs=pl.BlockSpec(memory_space=pl.ANY),
        out_shape=jax.ShapeDtypeStruct((rows, d_model), x.dtype),
        scratch_shapes=[
            pltpu.VMEM((rows, d_model), x.dtype),
            pltpu.VMEM((n_kv, d_model, gw), wq.dtype),
            pltpu.VMEM((n_kv, gw, d_model), wo.dtype),
            pltpu.VMEM((n_kv, batch, sk, dh), k_cache.dtype),
            pltpu.VMEM((n_kv, batch, sk, dh), v_cache.dtype),
            pltpu.VMEM((rows, d_model), jnp.float32),
            pltpu.VMEM((rows, d_model), x.dtype),
            pltpu.SemaphoreType.DMA((_NUM_SEMS,)),
        ],
        compiler_params=pltpu.CompilerParams(
            vmem_limit_bytes=48 * 1024 * 1024,
            flags={"XLA_TPU_RESCHEDULE_DMA_DONES": True},
        ),
    )(x.reshape(rows, d_model), k_cache, v_cache, wq, wo)
    return out.reshape(batch, sq, d_model)
```

```python
import functools

import jax
import jax.numpy as jnp
import jax.experimental.pallas as pl
import jax.experimental.pallas.tpu as pltpu

_LOG2E = 1.4426950408889634
_T = 128
_NUM_SEMS = 4
_N_PRO = 4
_NT_DIMS = (((1,), (1,)), ((), ()))
_TAIL_ROWS = (0, 256, 384, 448, 480, 496, 512)


def _copy_stages(rows):
    x = lambda k: ("x", k, 0, rows)
    w = lambda g, k: ("wqk", g, k)
    group = lambda g: [("k", g), ("wo", g - 1), ("v", g)]
    return [
        [w(0, 0), ("x", 0, 0, rows // 2)], [("x", 0, rows // 2, rows)],
        [w(1, 0)], [w(2, 0)], [w(3, 0)],
        [x(1), w(0, 1)], [w(1, 1)], [w(2, 1)], [w(3, 1)],
        [x(2), w(0, 2)], [w(1, 2)], [w(2, 2), w(3, 2)],
        [x(3), w(0, 3), w(1, 3)], [w(2, 3), w(3, 3)],
        [("k", 0), ("wq", 4), ("v", 0)],
        group(1) + [("wq", 5)],
        group(2) + [("wq", 6)],
        group(3) + [("wq", 7)],
        group(4) + group(5),
        group(6) + group(7) + [("wo", 7)],
    ]


def _schedule(n_kv):
    tasks = [("prologue",)]
    for g in range(n_kv):
        for j in range(4):
            tasks.append(("scores", g, j))
            tasks.append(("qproj", _N_PRO, j) if g == 0 else ("oproj", g - 1, j))
        nxt = _N_PRO + g
        if g >= 1 and nxt < n_kv:
            tasks += [("pv", g, 0), ("qproj", nxt, 0), ("qproj", nxt, 1),
                      ("pv", g, 1), ("qproj", nxt, 2), ("qproj", nxt, 3)]
        else:
            tasks += [("pv", g, 0), ("pv", g, 1)]
    tasks += [("oproj", n_kv - 1, j) for j in range(4)]
    return tasks


def _gqa_block_kernel(x_hbm, k_hbm, v_hbm, wq_hbm, wo_hbm, out_hbm,
                      xw_v, wo_v, k_v, v_v, acc_v, out_v, sems,
                      *, batch, sq, n_kv, rep, dh, scale):
    f32, bf16 = jnp.float32, jnp.bfloat16
    rows = batch * sq
    gw = rep * dh
    n_slabs = xw_v.shape[2] // _T
    stages = _copy_stages(rows)
    n_stages = len(stages)

    def copy(item, stage):
        sem = sems.at[stage % _NUM_SEMS]
        kind, g = item[0], item[1]
        if kind == "x":
            rws, cols = pl.ds(item[2], item[3] - item[2]), pl.ds(item[1] * _T, _T)
            return pltpu.make_async_copy(x_hbm.at[rws, cols], xw_v.at[0, rws, cols], sem)
        if kind == "wqk":
            rws = pl.ds(item[2] * _T, _T)
            return pltpu.make_async_copy(
                wq_hbm.at[rws, pl.ds(g * gw, gw)], xw_v.at[1 + g, rws, :], sem)
        if kind == "wq":
            return pltpu.make_async_copy(
                wq_hbm.at[:, pl.ds(g * gw, gw)], xw_v.at[1 + g], sem)
        if kind == "wo":
            return pltpu.make_async_copy(
                wo_hbm.at[pl.ds(g * gw, gw), :], wo_v.at[g], sem)
        if kind == "k":
            return pltpu.make_async_copy(k_hbm.at[:, g], k_v.at[g], sem)
        assert kind == "v", kind
        return pltpu.make_async_copy(v_hbm.at[:, g], v_v.at[g], sem)

    def start_stage(s):
        for item in stages[s]:
            copy(item, s).start()

    waited = []

    def wait_through(stage):
        while len(waited) <= stage:
            s = len(waited)
            for item in stages[s]:
                copy(item, s).wait()
            waited.append(s)
            if s + _NUM_SEMS < n_stages:
                start_stage(s + _NUM_SEMS)

    stage_of = {item: s for s, st in enumerate(stages) for item in st}

    def need(item):
        wait_through(stage_of[item])

    def need_x(k, r0, r1):
        wait_through(max(s for item, s in stage_of.items()
                         if item[:2] == ("x", k) and item[2] < r1 and item[3] > r0))

    q, p, o = {}, {}, {}
    out_copies = []

    def prologue():
        n_rb = 4
        acc = {}
        for k in range(n_slabs):
            ks = slice(k * _T, (k + 1) * _T)
            for g in range(_N_PRO):
                parts = []
                for i in range(n_rb):
                    r0, r1 = i * rows // n_rb, (i + 1) * rows // n_rb
                    need_x(k, r0, r1)
                    xi = xw_v[0, r0:r1, ks]
                    need(("wqk", g, k))
                    parts.append(jnp.dot(xi, xw_v[1 + g, ks, :], preferred_element_type=f32))
                part = jnp.concatenate(parts, axis=0)
                acc[g] = part if k == 0 else acc[g] + part
        for g in range(_N_PRO):
            for h in range(rep):
                q[g, h] = acc[g][:, h * dh:(h + 1) * dh]

    def qproj(g, h):
        need(("wq", g))
        q[g, h] = jnp.dot(xw_v[0], xw_v[1 + g, :, h * dh:(h + 1) * dh],
                          preferred_element_type=f32)

    def scores(g, j):
        need(("k", g))
        for b in (2 * j, 2 * j + 1):
            qs = jnp.concatenate(
                [q[g, h][b * sq:(b + 1) * sq] for h in range(rep)], axis=0).astype(bf16)
            st = jax.lax.dot_general(k_v[g, b], qs, _NT_DIMS,
                                     preferred_element_type=f32)
            m = jnp.max(st, axis=0, keepdims=True)
            e = jnp.exp2((st - m) * (scale * _LOG2E))
            denom = jnp.sum(e, axis=0, keepdims=True)
            p[g, b] = (e * pl.reciprocal(denom, approx=False)).astype(bf16).T

    def pv(g, half):
        need(("v", g))
        for b in range(half * batch // 2, (half + 1) * batch // 2):
            ob = jnp.dot(p.pop((g, b)), v_v[g, b], preferred_element_type=f32)
            o[g, b] = jnp.concatenate(
                [ob[h * sq:(h + 1) * sq] for h in range(rep)], axis=1)

    def oproj(g, j):
        need(("wo", g))
        if j == 0:
            o[g] = jnp.concatenate([o.pop((g, b)) for b in range(batch)], axis=0)
        cols = slice(j * _T, (j + 1) * _T)
        if g < n_kv - 1:
            part = jnp.dot(o[g].astype(bf16), wo_v[g, :, cols], preferred_element_type=f32)
            if g == 0:
                acc_v[:, cols] = part
            else:
                acc_v[:, cols] += part
            return
        wait_through(n_stages - 1)
        bounds = _TAIL_ROWS if j == 3 else (0, rows)
        for r0, r1 in zip(bounds[:-1], bounds[1:]):
            rws = slice(r0, r1)
            part = jnp.dot(o[g][rws].astype(bf16), wo_v[g, :, cols],
                           preferred_element_type=f32)
            out_v[rws, cols] = (acc_v[rws, cols] + part).astype(out_v.dtype)
            out_copy = pltpu.make_async_copy(
                out_v.at[rws, cols], out_hbm.at[rws, cols], sems.at[n_stages % _NUM_SEMS])
            out_copy.start()
            out_copies.append(out_copy)

    for s in range(_NUM_SEMS):
        start_stage(s)
    run = dict(prologue=prologue, qproj=qproj, scores=scores, pv=pv, oproj=oproj)
    for task in _schedule(n_kv):
        run[task[0]](*task[1:])
    for out_copy in out_copies:
        out_copy.wait()


@jax.jit
def pallas_standalone__gqa_block_cached__near_ridge_kernel(
    x: jax.Array,
    k_cache: jax.Array,
    v_cache: jax.Array,
    wq: jax.Array,
    wo: jax.Array,
):
    batch, sq, d_model = x.shape
    _, n_kv, sk, dh = k_cache.shape
    n_q = wq.shape[1] // dh
    rep = n_q // n_kv
    gw = rep * dh
    rows = batch * sq
    assert (batch, sq, d_model, n_kv, sk, dh, n_q) == (8, 64, 512, 8, 64, 128, 32)

    kernel = functools.partial(
        _gqa_block_kernel, batch=batch, sq=sq, n_kv=n_kv, rep=rep, dh=dh,
        scale=dh ** -0.5)
    out = pl.pallas_call(
        kernel,
        in_specs=[pl.BlockSpec(memory_space=pl.ANY)] * 5,
        out_specs=pl.BlockSpec(memory_space=pl.ANY),
        out_shape=jax.ShapeDtypeStruct((rows, d_model), x.dtype),
        scratch_shapes=[
            pltpu.VMEM((1 + n_kv, d_model, gw), x.dtype),
            pltpu.VMEM((n_kv, gw, d_model), wo.dtype),
            pltpu.VMEM((n_kv, batch, sk, dh), k_cache.dtype),
            pltpu.VMEM((n_kv, batch, sk, dh), v_cache.dtype),
            pltpu.VMEM((rows, d_model), jnp.float32),
            pltpu.VMEM((rows, d_model), x.dtype),
            pltpu.SemaphoreType.DMA((_NUM_SEMS,)),
        ],
        compiler_params=pltpu.CompilerParams(
            vmem_limit_bytes=64 * 1024 * 1024,
            flags={"XLA_TPU_RESCHEDULE_DMA_DONES": True},
        ),
    )(x.reshape(rows, d_model), k_cache, v_cache, wq, wo)
    return out.reshape(batch, sq, d_model)
```

```python
import functools

import jax
import jax.numpy as jnp
import jax.experimental.pallas as pl
import jax.experimental.pallas.tpu as pltpu

_LOG2E = 1.4426950408889634
_T = 128
_NUM_SEMS = 6
_N_PRO = 4
_NT_DIMS = (((1,), (1,)), ((), ()))
_TAIL_ROWS = (0, 256, 384, 448, 480, 496, 512)


def _copy_stages(rows):
    x = lambda k: ("x", k, 0, rows)
    w = lambda g, k: ("wqk", g, k)
    group = lambda g: [("k", g), ("wo", g - 1), ("v", g)]
    return [
        [w(0, 0)],
        [("x", 0, 0, rows // 4)], [("x", 0, rows // 4, rows // 2)],
        [("x", 0, rows // 2, rows)],
        [w(1, 0)], [w(2, 0)], [w(3, 0)],
        [x(1), w(0, 1)], [w(1, 1)], [w(2, 1)], [w(3, 1)],
        [x(2), w(0, 2)], [w(1, 2)], [w(2, 2), w(3, 2)],
        [x(3), w(0, 3), w(1, 3)], [w(2, 3), w(3, 3)],
        [("k", 0), ("wq", 4), ("v", 0)],
        group(1) + [("wq", 5)],
        group(2) + [("wq", 6)],
        group(3) + [("wq", 7)],
        group(4) + group(5),
        group(6) + group(7) + [("wo", 7)],
    ]


def _schedule(n_kv):
    tasks = [("prologue",)]
    for g in range(n_kv):
        for j in range(4):
            tasks.append(("scores", g, j))
            tasks.append(("qproj", _N_PRO, j) if g == 0 else ("oproj", g - 1, j))
        nxt = _N_PRO + g
        if g >= 1 and nxt < n_kv:
            tasks += [("pv", g, 0), ("qproj", nxt, 0), ("qproj", nxt, 1),
                      ("pv", g, 1), ("qproj", nxt, 2), ("qproj", nxt, 3)]
        else:
            tasks += [("pv", g, 0), ("pv", g, 1)]
    tasks += [("oproj", n_kv - 1, j) for j in range(4)]
    return tasks


def _gqa_block_body(x_hbm, k_hbm, v_hbm, wq_hbm, wo_hbm, out_hbm,
                    xw_v, wo_v, k_v, v_v, acc_v, out_v, sems,
                    *, batch, sq, n_kv, rep, dh, scale):
    f32, bf16 = jnp.float32, jnp.bfloat16
    rows = batch * sq
    gw = rep * dh
    n_slabs = xw_v.shape[2] // _T
    stages = _copy_stages(rows)
    n_stages = len(stages)

    def copy(item, stage):
        sem = sems.at[stage % _NUM_SEMS]
        kind, g = item[0], item[1]
        if kind == "x":
            rws, cols = pl.ds(item[2], item[3] - item[2]), pl.ds(item[1] * _T, _T)
            return pltpu.make_async_copy(x_hbm.at[rws, cols], xw_v.at[0, rws, cols], sem)
        if kind == "wqk":
            rws = pl.ds(item[2] * _T, _T)
            return pltpu.make_async_copy(
                wq_hbm.at[rws, pl.ds(g * gw, gw)], xw_v.at[1 + g, rws, :], sem)
        if kind == "wq":
            return pltpu.make_async_copy(
                wq_hbm.at[:, pl.ds(g * gw, gw)], xw_v.at[1 + g], sem)
        if kind == "wo":
            return pltpu.make_async_copy(
                wo_hbm.at[pl.ds(g * gw, gw), :], wo_v.at[g], sem)
        if kind == "k":
            return pltpu.make_async_copy(k_hbm.at[:, g], k_v.at[g], sem)
        assert kind == "v", kind
        return pltpu.make_async_copy(v_hbm.at[:, g], v_v.at[g], sem)

    def start_stage(s):
        for item in stages[s]:
            copy(item, s).start()

    waited = []

    def wait_through(stage):
        while len(waited) <= stage:
            s = len(waited)
            for item in stages[s]:
                copy(item, s).wait()
            waited.append(s)
            if s + _NUM_SEMS < n_stages:
                start_stage(s + _NUM_SEMS)

    stage_of = {item: s for s, st in enumerate(stages) for item in st}

    def need(item):
        wait_through(stage_of[item])

    def need_x(k, r0, r1):
        wait_through(max(s for item, s in stage_of.items()
                         if item[:2] == ("x", k) and item[2] < r1 and item[3] > r0))

    q, p, o = {}, {}, {}
    out_copies = []

    def prologue():
        n_rb = 4
        acc = {}
        for k in range(n_slabs):
            ks = slice(k * _T, (k + 1) * _T)
            for g in range(_N_PRO):
                parts = []
                for i in range(n_rb):
                    r0, r1 = i * rows // n_rb, (i + 1) * rows // n_rb
                    need(("wqk", g, k))
                    w = xw_v[1 + g, ks, :]
                    need_x(k, r0, r1)
                    parts.append(jnp.dot(xw_v[0, r0:r1, ks], w, preferred_element_type=f32))
                part = jnp.concatenate(parts, axis=0)
                acc[g] = part if k == 0 else acc[g] + part
        for g in range(_N_PRO):
            for h in range(rep):
                q[g, h] = acc[g][:, h * dh:(h + 1) * dh]

    def qproj(g, h):
        need(("wq", g))
        q[g, h] = jnp.dot(xw_v[0], xw_v[1 + g, :, h * dh:(h + 1) * dh],
                          preferred_element_type=f32)

    def scores(g, j):
        need(("k", g))
        for b in (2 * j, 2 * j + 1):
            qs = jnp.concatenate(
                [q[g, h][b * sq:(b + 1) * sq] for h in range(rep)], axis=0).astype(bf16)
            st = jax.lax.dot_general(k_v[g, b], qs, _NT_DIMS,
                                     preferred_element_type=f32)
            m = jnp.max(st, axis=0, keepdims=True)
            e = jnp.exp2((st - m) * (scale * _LOG2E))
            denom = jnp.sum(e, axis=0, keepdims=True)
            p[g, b] = (e * pl.reciprocal(denom, approx=False)).astype(bf16).T

    def pv(g, half):
        need(("v", g))
        for b in range(half * batch // 2, (half + 1) * batch // 2):
            ob = jnp.dot(p.pop((g, b)), v_v[g, b], preferred_element_type=f32)
            o[g, b] = jnp.concatenate(
                [ob[h * sq:(h + 1) * sq] for h in range(rep)], axis=1)

    def oproj(g, j):
        need(("wo", g))
        if j == 0:
            o[g] = jnp.concatenate([o.pop((g, b)) for b in range(batch)], axis=0)
        cols = slice(j * _T, (j + 1) * _T)
        if g < n_kv - 1:
            part = jnp.dot(o[g].astype(bf16), wo_v[g, :, cols], preferred_element_type=f32)
            if g == 0:
                acc_v[:, cols] = part
            else:
                acc_v[:, cols] += part
            return
        wait_through(n_stages - 1)
        bounds = _TAIL_ROWS if j == 3 else (0, rows)
        for r0, r1 in zip(bounds[:-1], bounds[1:]):
            rws = slice(r0, r1)
            part = jnp.dot(o[g][rws].astype(bf16), wo_v[g, :, cols],
                           preferred_element_type=f32)
            out_v[rws, cols] = (acc_v[rws, cols] + part).astype(out_v.dtype)
            out_copy = pltpu.make_async_copy(
                out_v.at[rws, cols], out_hbm.at[rws, cols], sems.at[n_stages % _NUM_SEMS])
            out_copy.start()
            out_copies.append(out_copy)

    for s in range(_NUM_SEMS):
        start_stage(s)
    run = dict(prologue=prologue, qproj=qproj, scores=scores, pv=pv, oproj=oproj)
    for task in _schedule(n_kv):
        run[task[0]](*task[1:])
    for out_copy in out_copies:
        out_copy.wait()


def _gqa_block_kernel(*refs, **sizes):
    pl.run_scoped(
        functools.partial(_gqa_block_body, *refs, **sizes),
        pltpu.SemaphoreType.DMA((_NUM_SEMS,)),
    )


@jax.jit
def pallas_standalone__gqa_block_cached__near_ridge_kernel(
    x: jax.Array,
    k_cache: jax.Array,
    v_cache: jax.Array,
    wq: jax.Array,
    wo: jax.Array,
):
    batch, sq, d_model = x.shape
    _, n_kv, sk, dh = k_cache.shape
    n_q = wq.shape[1] // dh
    rep = n_q // n_kv
    gw = rep * dh
    rows = batch * sq
    assert (batch, sq, d_model, n_kv, sk, dh, n_q) == (8, 64, 512, 8, 64, 128, 32)

    kernel = functools.partial(
        _gqa_block_kernel, batch=batch, sq=sq, n_kv=n_kv, rep=rep, dh=dh,
        scale=dh ** -0.5)
    out = pl.pallas_call(
        kernel,
        in_specs=[pl.BlockSpec(memory_space=pl.ANY)] * 5,
        out_specs=pl.BlockSpec(memory_space=pl.ANY),
        out_shape=jax.ShapeDtypeStruct((rows, d_model), x.dtype),
        scratch_shapes=[
            pltpu.VMEM((1 + n_kv, d_model, gw), x.dtype),
            pltpu.VMEM((n_kv, gw, d_model), wo.dtype),
            pltpu.VMEM((n_kv, batch, sk, dh), k_cache.dtype),
            pltpu.VMEM((n_kv, batch, sk, dh), v_cache.dtype),
            pltpu.VMEM((rows, d_model), jnp.float32),
            pltpu.VMEM((rows, d_model), x.dtype),
        ],
        compiler_params=pltpu.CompilerParams(
            vmem_limit_bytes=64 * 1024 * 1024,
            flags={"XLA_TPU_RESCHEDULE_DMA_DONES": True},
        ),
    )(x.reshape(rows, d_model), k_cache, v_cache, wq, wo)
    return out.reshape(batch, sq, d_model)
```
